```python
import os as _os
_os.environ.setdefault("JAX_PLATFORMS", "cpu")
import jax
import jax.numpy as jnp

def _softmax(x, axis=-1):
    return jax.nn.softmax(x, axis=axis)
def _gelu(x):
    return jax.nn.gelu(x, approximate=True)
def _silu(x):
    return jax.nn.silu(x)
def _sigmoid(x):
    return jax.nn.sigmoid(x)
def _layernorm(x, axis=-1, eps=1e-5):
    m = jnp.mean(x, axis=axis, keepdims=True)
    v = jnp.var(x, axis=axis, keepdims=True)
    return (x - m) / jnp.sqrt(v + eps)
def _scatter_add(tgt, idx, src, axis=0):
    return tgt.at[idx].add(src)
def _segment_sum(src, seg, n):
    return jax.ops.segment_sum(src, seg, n)
class _Rng:
    def __init__(self, key):
        self._k = key
    def _next(self):
        self._k, sub = jax.random.split(self._k)
        return sub
    def normal(self, shape):
        return jax.random.normal(self._next(), shape, dtype=jnp.bfloat16)
    def randint(self, lo, hi, shape):
        return jax.random.randint(self._next(), shape, lo, hi, dtype=jnp.int32)
    def uniform(self, shape, lo=0.0, hi=1.0):
        return jax.random.uniform(self._next(), shape, jnp.bfloat16, lo, hi)
    def permutation(self, n):
        return jax.random.permutation(self._next(), n)


kernel_name = 'gated_mix__grouped_kv_mqa__glu_gated_reglu__prompt'

def setup_inputs():
    _rng = _Rng(jax.random.key(int.from_bytes(__import__("os").urandom(4), "little")))
    _w = (lambda a: (lambda t: t.astype(jnp.bfloat16) if jnp.issubdtype(t.dtype, jnp.floating) else t)(jnp.asarray(a)))
    def _A_setup():
        B, S, D, H = 1, 2048, 640, 32
        Dh = D // H
        return {
            "x": _w((lambda *s: _rng.normal(s) * 0.05)(B, S, D)),
            "wq": _w((lambda *s: _rng.normal(s) * 0.2)(D, H * Dh)),
            "wk": _w((lambda *s: _rng.normal(s) * 0.2)(D, Dh)),
            "wv": _w((lambda *s: _rng.normal(s) * 0.05)(D, Dh)),
            "wo": _w((lambda *s: _rng.normal(s) * 0.05)(H * Dh, D)),
        }
    _A_in = _A_setup()

    def _B_setup():
        B, S, D, F = 1, 2048, 640, 1536
        return {
            "x": _w((lambda *s: _rng.normal(s) * 0.05)(B, S, D)),
            "W_gate": _w((lambda *s: _rng.normal(s) * 0.4)(D, F) * (2.0 / D) ** 0.5),
            "W_up": _w((lambda *s: _rng.normal(s) * 0.4)(D, F) * (2.0 / D) ** 0.5),
            "W_down": _w((lambda *s: _rng.normal(s) * 0.4)(F, D) * (1.0 / F) ** 0.5),
        }
    _B_in = _B_setup()

    return {
        "A_x": _A_in["x"],
        "A_wq": _A_in["wq"],
        "A_wk": _A_in["wk"],
        "A_wv": _A_in["wv"],
        "A_wo": _A_in["wo"],
        "B_x": _B_in["x"],
        "B_W_gate": _B_in["W_gate"],
        "B_W_up": _B_in["W_up"],
        "B_W_down": _B_in["W_down"],
        "gate_w": _w((lambda *s: _rng.normal(s) * 0.05)(640) * 16.0),
    }

def reference(A_x, A_wq, A_wk, A_wv, A_wo, B_x, B_W_gate, B_W_up, B_W_down, gate_w):
    def _A_ref(x, wq, wk, wv, wo):
        B, S, D = x.shape
        H = 32
        Dh = D // H
        q = (lambda x, *d: x.transpose(*d))((x @ wq).reshape(B, S, H, Dh), 0, 2, 1, 3)
        k = x @ wk
        v = x @ wv
        scores = jnp.einsum("bhqd,bkd->bhqk", q, k) * (Dh ** -0.5)
        p = _softmax(scores, axis=-1)
        o = jnp.einsum("bhqk,bkd->bhqd", p, v)
        return (lambda x, *d: x.transpose(*d))(o, 0, 2, 1, 3).reshape(B, S, H * Dh) @ wo

    def _B_ref(x, W_gate, W_up, W_down):
        gate = jnp.einsum("bsd,df->bsf", x, W_gate)
        up = jnp.einsum("bsd,df->bsf", x, W_up)
        gate = gate * (lambda x, dt: x.astype(dt))(gate > 0, gate.dtype)
        h = gate * up
        return jnp.einsum("bsf,fd->bsd", h, W_down)

    x = A_x
    g = _sigmoid((x * gate_w).sum(-1, keepdims=True))
    a = _A_ref(x, A_wq, A_wk, A_wv, A_wo)
    b = _B_ref(x, B_W_gate, B_W_up, B_W_down)
    return g * a + (1 - g) * b
```

```python
import functools
import math

import jax
import jax.numpy as jnp
from jax import lax
import jax.experimental.pallas as pl
import jax.experimental.pallas.tpu as pltpu

F32 = jnp.float32
BF16 = jnp.bfloat16
NN = (((1,), (0,)), ((), ()))
NT = (((1,), (1,)), ((), ()))
TN = (((0,), (0,)), ((), ()))


def _dot(a, b, dims=NN):
    return lax.dot_general(a, b, dims, preferred_element_type=F32)


def make(S=2048, D=640, H=32, F=1536, QB=512, CK=256, LAG=1, PAIRS=1, PF32=False, ONLINE=True,
         flags=None, name="gm"):
    DH = D // H
    NQB = S // QB
    NC = S // CK
    MV = 24
    KP = 32
    pdt = F32 if PF32 else BF16
    qscale = (DH ** -0.5) * math.log2(math.e)

    def kernel(x_hbm, wq_hbm, wkt_hbm, wvt_hbm, wo_hbm, wg_hbm, wu_hbm, wd_hbm, gw_ref, out_hbm,
               x_v, wq_v, wkt_v, wvt_v, wo_v, wg_v, wu_v, wd_v, k_s, vt_s, gc_s, gr_s, qt_s, ot_s, out_v,
               sems, osems):
        cps = [
            pltpu.make_async_copy(wkt_hbm, wkt_v, sems.at[0]),
            pltpu.make_async_copy(wvt_hbm, wvt_v, sems.at[1]),
            pltpu.make_async_copy(x_hbm, x_v, sems.at[2]),
            pltpu.make_async_copy(wq_hbm, wq_v, sems.at[3]),
            pltpu.make_async_copy(wg_hbm, wg_v, sems.at[4]),
            pltpu.make_async_copy(wu_hbm, wu_v, sems.at[5]),
            pltpu.make_async_copy(wd_hbm, wd_v, sems.at[6]),
            pltpu.make_async_copy(wo_hbm, wo_v, sems.at[7]),
        ]
        for c in cps:
            c.start()
        cps[0].wait()
        cps[1].wait()
        cps[2].wait()

        zpad = jnp.zeros((MV - DH, D), F32)
        gw = gw_ref[...].astype(F32).reshape(1, D)
        w_small = jnp.concatenate(
            [wkt_v[...].astype(F32), zpad, wvt_v[...].astype(F32), zpad,
             jnp.broadcast_to(gw, (8, D))], axis=0)
        kvg = _dot(w_small, x_v[...], NT)
        row = lax.broadcasted_iota(jnp.int32, (MV, S), 0)
        vt = kvg[MV:2 * MV].astype(BF16).astype(F32)
        vt_s[...] = jnp.where(row == DH, 1.0, vt)
        g = jax.nn.sigmoid(kvg[2 * MV:2 * MV + 8])
        gr_s[...] = g
        kp = jnp.concatenate([kvg[:MV], jnp.zeros((128 - MV, S), F32)], axis=0)
        k_s[...] = kp.T[:, :KP].astype(BF16)
        gc_s[...] = jnp.broadcast_to(1.0 - g[0:1], (128, S)).T
        cps[3].wait()

        def attend(q):
            ss = {}
            acc = None
            m = None
            for i in range(NC + LAG):
                if i < NC:
                    ss[i] = _dot(k_s[i * CK:(i + 1) * CK, :], q)
                j = i - LAG
                if j >= 0:
                    s = ss.pop(j)
                    if ONLINE:
                        mc = jnp.max(jnp.max(s.reshape(CK // 8, 8, QB), axis=0), axis=0, keepdims=True)
                        m_new = mc if m is None else jnp.maximum(m, mc)
                        p = jnp.exp2(s - m_new).astype(pdt)
                        d = _dot(vt_s[:, j * CK:(j + 1) * CK], p)
                        acc = d if acc is None else acc * jnp.exp2(m - m_new) + d
                        m = m_new
                    else:
                        p = jnp.exp2(s).astype(pdt)
                        d = _dot(vt_s[:, j * CK:(j + 1) * CK], p)
                        acc = d if acc is None else acc + d
            return acc

        def qblock(qb, carry):
            r0 = pl.multiple_of(qb * QB, QB)
            xb = x_v[pl.ds(r0, QB), :]
            q = _dot(xb, wq_v[...]) * qscale
            qt_s[...] = q.T.reshape(H // 2, 2 * DH, QB)
            grow = gr_s[0:1, pl.ds(r0, QB)]

            def pair(hp, c):
                for u in range(PAIRS):
                    idx = hp * PAIRS + u
                    qp = qt_s[idx]
                    z = jnp.zeros((KP - DH, QB), F32)
                    outs = []
                    for e in range(2):
                        qh = jnp.concatenate([qp[e * DH:(e + 1) * DH], z], axis=0).astype(BF16)
                        acc = attend(qh)
                        outs.append(acc[:DH] * (grow / acc[DH:DH + 1]))
                    ot_s[idx] = jnp.concatenate(outs, axis=0)
                return c

            lax.fori_loop(0, H // 2 // PAIRS, pair, 0)

            @pl.when(qb == 0)
            def _():
                for c in cps[4:]:
                    c.wait()

            a = _dot(ot_s[...].reshape(D, QB).astype(BF16), wo_v[...], TN)
            xb = x_v[pl.ds(r0, QB), :]
            gate = _dot(xb, wg_v[...])
            up = _dot(xb, wu_v[...])
            hh = (jnp.where(gate > 0, gate, gate * 0.0) * up).astype(BF16)
            b = _dot(hh, wd_v[...])
            gc = gc_s[pl.ds(r0, QB), :]
            out_v[qb] = (a + jnp.tile(gc, (1, D // 128)) * b).astype(out_v.dtype)
            pltpu.make_async_copy(out_v.at[qb], out_hbm.at[pl.ds(r0, QB)], osems.at[qb]).start()
            return carry

        lax.fori_loop(0, NQB, qblock, 0)
        for i in range(NQB):
            pltpu.make_async_copy(out_v.at[i], out_hbm.at[pl.ds(i * QB, QB)], osems.at[i]).wait()

    anyspec = pl.BlockSpec(memory_space=pl.ANY)
    call = pl.pallas_call(
        kernel,
        out_shape=jax.ShapeDtypeStruct((S, D), BF16),
        in_specs=[anyspec] * 8 + [pl.BlockSpec(memory_space=pltpu.VMEM)],
        out_specs=anyspec,
        scratch_shapes=[
            pltpu.VMEM((S, D), BF16), pltpu.VMEM((D, D), BF16), pltpu.VMEM((DH, D), BF16),
            pltpu.VMEM((DH, D), BF16), pltpu.VMEM((D, D), BF16), pltpu.VMEM((D, F), BF16),
            pltpu.VMEM((D, F), BF16), pltpu.VMEM((F, D), BF16),
            pltpu.VMEM((S, KP), BF16), pltpu.VMEM((MV, S), F32), pltpu.VMEM((S, 128), F32),
            pltpu.VMEM((8, S), F32),
            pltpu.VMEM((H // 2, 2 * DH, QB), F32), pltpu.VMEM((H // 2, 2 * DH, QB), F32),
            pltpu.VMEM((NQB, QB, D), BF16),
            pltpu.SemaphoreType.DMA((8,)), pltpu.SemaphoreType.DMA((NQB,)),
        ],
        compiler_params=pltpu.CompilerParams(vmem_limit_bytes=100 * 2**20, flags=flags),
        name=name,
    )

    @jax.jit
    def fn(A_x, A_wq, A_wk, A_wv, A_wo, B_x, B_W_gate, B_W_up, B_W_down, gate_w):
        out = call(A_x.reshape(S, D), A_wq, A_wk.T, A_wv.T, A_wo, B_W_gate, B_W_up, B_W_down, gate_w)
        return out.reshape(1, S, D)

    return fn


_fn = make(PF32=True)


@jax.jit
def pallas_gated_mix__grouped_kv_mqa__glu_gated_reglu__prompt_kernel(
    A_x, A_wq, A_wk, A_wv, A_wo, B_x, B_W_gate, B_W_up, B_W_down, gate_w):
    return _fn(A_x, A_wq, A_wk, A_wv, A_wo, B_x, B_W_gate, B_W_up, B_W_down, gate_w)
```

```python
import math

import jax
import jax.numpy as jnp
from jax import lax
import jax.experimental.pallas as pl
import jax.experimental.pallas.tpu as pltpu

F32 = jnp.float32
BF16 = jnp.bfloat16
U32 = jnp.uint32
NN = (((1,), (0,)), ((), ()))
NT = (((1,), (1,)), ((), ()))


def _dot(a, b, dims=NN):
    return lax.dot_general(a, b, dims, preferred_element_type=F32)


def _bits(v):
    return pltpu.bitcast(v, U32)


def make(S=2048, D=640, H=32, F=1536, NB=28, NPRE=4, LAT=152, FWD=200, LEAD=60, SH=14, TAILR=2,
         QMAX=8, DLY=150, MODE='-rmrmmr', KB0=6, EARLY=0, WOFF=0.5, SMALL=1, ITER=None, SLOTS=(6, 6),  SHIFT=None, FW=None, FALLBACK=True,
         flags=None, name="gm", verbose=False, info=None):
    T = 128
    DH = D // H
    HD = DH // 2
    NBLK = S // T
    NC = S // T
    NU = H // 4
    MV = 24
    KP = 32
    ND = D // T
    NF = F // T
    XC = 512
    NXC = S // XC
    NSB = NB // 2
    NP = 7
    qscale = (DH ** -0.5) * math.log2(math.e)

    nb = [((c + 1) * NB) // NC - (c * NB) // NC for c in range(NC)]
    npre = [0] * NC
    for _ in range(NPRE):
        npre[min(range(NC), key=lambda c: (nb[c] + npre[c], c))] += 1
    ng = [8 - a - b for a, b in zip(nb, npre)]
    b0, p0, g0 = ([sum(v[:c]) for c in range(NC)] for v in (nb, npre, ng))
    vgrp = [(b // 16) * 16 + (b % 2) * 8 + (b % 16) // 2 for b in range(NB)]
    rest = [g for g in range(S // 16) if g not in vgrp]
    pgrp, mgrp = rest[:NPRE], rest[NPRE:]
    assert max(vgrp + pgrp) < XC // 16
    order = []
    for c in range(NC):
        extra = [("v", b0[c] + a) for a in range(nb[c])] + [("p", p0[c] + a) for a in range(npre[c])]
        seq = [("m", g0[c] + a) for a in range(ng[c])]
        for e, at in reversed(list(zip(extra, SLOTS))):
            seq.insert(at, e)
        order.append(seq)

    RING = 16
    sizes = dict(sv=8 * RING, keep=16, k=len(mgrp), v=3 * NC, x=8 * ND * NBLK)
    base, top = {}, 0
    for key, n in sizes.items():
        base[key] = top
        top += -(-n // 4) * 4
    base["h"] = base["k"]
    base["o"] = base["h"] + 16 * NF
    top2 = base["o"] + 16 * ND

    oproj = [("ob",)] + [("oa", n) for n in range(4)] + [("oc",), ("oa", 4)]
    ffn = []
    for c in range(NF // 2):
        ffn += [("gu_b", c), ("gate", 2 * c), ("up", 2 * c), ("gate", 2 * c + 1), ("up", 2 * c + 1)]
        if c == 0:
            ffn += oproj
        if c % 2 == 1:
            ffn += [("down", c // 2, n) for n in range(ND)]
    NUS = NU // SMALL
    ffn = ffn[len(ffn) - len(ffn) // SMALL - (SMALL > 1):]
    tail = ffn[len(ffn) - TAILR:]
    ffn = ffn[:len(ffn) - TAILR]
    prog = []
    nt = NUS * NC
    stream = [(t, a) for t in range(nt) for a in range(ng[t % NC])]
    now, pend, si, wi = 0, [], 0, 0
    while si < len(stream) or pend:
        if pend and now - pend[0][1] >= (LAT if si < len(stream) else T):
            prog.append(("pv", pend.pop(0)[0]))
            now += MV
            if wi < len(ffn) and (wi + WOFF) * len(stream) <= si * len(ffn):
                prog.append(ffn[wi])
                now += 32 if ffn[wi][0] == "oc" else T
                wi += 1
        elif si < len(stream):
            t, a = stream[si]
            last = prog[-1] if prog else ("",)
            if last[0] == "qk" and last[1] == t // NC and len(last[2]) < QMAX:
                last[2].append(g0[t % NC] + a)
            else:
                prog.append(("qk", t // NC, [g0[t % NC] + a]))
            si += 1
            now += 16
            if a == ng[t % NC] - 1:
                pend.append((t, now))
        else:
            if wi < len(ffn):
                prog.append(ffn[wi])
                wi += 1
            elif tail:
                prog.append(tail.pop(0))
            now += T
    prog += ffn[wi:] + tail

    when, now = [], 0
    for op in prog:
        n, cyc = {"qk": (len(op[-1]) if op[0] == "qk" else 0, 16), "pv": (3, 8), "oc": (1, 32),
                  "down": (16, 8), "oa": (16, 8), "ob": (16, 8)}.get(op[0], (8, 16))
        when.append([now + cyc * a for a in range(n)])
        now += cyc * n
    NPIECE = NUS * NSB * NP
    loads = [(tm, op) for op, row in zip(prog, when) for tm in row]
    pos = {op: i for i, op in enumerate(prog) if op[0] == "pv"}
    need = [(t // NC) * NSB * NP + (b0[t % NC] + nb[t % NC] + 1) // 2 * NP for t in range(nt)]
    assert all(SH + NPIECE * (when[pos["pv", t]][0] - LEAD) / loads[-1][0] >= need[t] for t in range(nt))
    pin, a = [], 0
    for n in range(NPIECE):
        while loads[a][0] * NPIECE < (n + 1) * loads[-1][0]:
            a += 1
        pin.append(a)
    if SHIFT:
        pin = sorted(min(max(p + s, 0), len(loads) - 1) for p, s in zip(pin, SHIFT))
    due = {tm: SH + sum(p <= a for p in pin) for a, (tm, _) in enumerate(loads)}
    second_ops = ("down", "oa", "ob", "oc")
    second = {(n + SH) % NPIECE: loads[p][1][0] in second_ops for n, p in enumerate(pin)}
    assert all(due[when[pos["pv", t]][0] ] >= need[t] for t in range(nt))
    if verbose:
        print(" ".join(op[0] + (str(len(op[2])) if op[0] == "qk" else "") for op in prog))
    if info is not None:
        info.update(pin=pin, loads=[tm for tm, _ in loads], total=now, kinds=[op[0] for _, op in loads])
        return None
    NZ = 64
    KR = (NP * HD - KB0) // NXC
    assert KB0 + NXC * KR == NP * HD

    def kernel(x_hbm, wq_hbm, wkt_hbm, wvt_hbm, wo_hbm, wg_hbm, wu_hbm, wd_hbm, gw_ref, out_hbm,
               x_v, wq_v, wkt_v, wvt_v, wo_v, wg_v, wu_v, wd_v,
               op_s, ho_s, kb_s, kt_s, kop_s, kpre_s, qt_s, qw_s, pre_s, gc_s, ot_s, acc0_s, acc1_s, gu_s, rg_s, b_s, c_s, out_v,
               zs, xsems, sems, wsems, osems):
        small = [pltpu.make_async_copy(wkt_hbm, wkt_v, sems.at[0]),
                 pltpu.make_async_copy(wvt_hbm, wvt_v, sems.at[1])]
        wq_cp = [pltpu.make_async_copy(wq_hbm.at[:, pl.ds(j * T, T)], wq_v.at[j], sems.at[2 + j]) for j in range(ND)]
        x_cp = [pltpu.make_async_copy(x_hbm.at[pl.ds(i * XC, XC)], x_v.at[i], xsems.at[i]) for i in range(NXC)]
        w_cp = []
        for src, dst, n in ((wg_hbm, wg_v, NF), (wu_hbm, wu_v, NF), (wd_hbm, wd_v, ND), (wo_hbm, wo_v, ND)):
            for j in range(n):
                w_cp.append(pltpu.make_async_copy(src.at[:, pl.ds(j * T, T)], dst.at[j], wsems.at[len(w_cp)]))
        for c in small + [x_cp[0]] + wq_cp:
            c.start()
        ot_s[...] = jnp.zeros(ot_s.shape, F32)
        b_s[:ND] = jnp.zeros((ND, T, T), F32)
        for i in range(NZ):
            zs[i] = 0
        for c in small:
            c.wait()

        def put(at, v):
            v = _bits(v)
            op_s[pl.ds(at, v.shape[0] // 8)] = v.reshape(v.shape[0] // 8, 8, T)

        def small_weights():
            zpad = jnp.zeros((MV - DH, D), F32)
            gw = gw_ref[...].astype(F32).reshape(1, D)
            return jnp.concatenate(
                [wkt_v[...].astype(F32), zpad, wvt_v[...].astype(F32), zpad,
                 jnp.broadcast_to(gw, (8, D))], axis=0)

        def key_rows(kt):
            return jnp.concatenate([kt, jnp.zeros((T - MV, kt.shape[1]), F32)], axis=0).T

        x_cp[0].wait()
        kt_s[...] = _dot(small_weights()[:MV], x_v[0], NT).astype(BF16).astype(F32)

        NKB = pl.cdiv(NSB, 8)
        lo = jnp.concatenate([kt_s[:, 2 * c * T:(2 * c + 1) * T] for c in range(NKB)], axis=1)
        hi = jnp.concatenate([kt_s[:, (2 * c + 1) * T:(2 * c + 2) * T] for c in range(NKB)], axis=1)
        a11, a12, a21, a22 = lo[:HD], lo[HD:DH], hi[:HD], hi[HD:DH]
        s1 = a21 + a22
        s2 = s1 - a11
        kop = jnp.concatenate([a11, a12, s2, a11 - a21, a22, s1, a12 - s2], axis=0)
        for i in range(NXC):
            kop_s[i] = kop[KB0 + KR * i:KB0 + KR * (i + 1)]

        def broadcast_keys(at, row):
            for c in range(NKB):
                nblk = min(8, NSB - 8 * c)
                col = jnp.broadcast_to(row[:, c * T:(c + 1) * T], (T, T)).T
                kb_s[8 * c:8 * c + nblk, at] = col[:16 * nblk].reshape(nblk, 16, T)

        if NPRE:
            k0 = key_rows(kt_s[...])
            kpre_s[...] = _bits(jnp.concatenate([k0[16 * g:16 * (g + 1)] for g in pgrp], axis=0).astype(BF16))
        for r in range(KB0):
            broadcast_keys(r, kop[r:r + 1])
        for c in wq_cp:
            c.wait()
        for c in x_cp[1:] + w_cp[:EARLY]:
            c.start()

        def queries(i, norm):
            @pl.when(i == 1)
            def _():
                for c in x_cp[1:]:
                    c.wait()
                for c in w_cp[EARLY:]:
                    c.start()

            def project(r):
                xb = x_v[i, r * T:(r + 1) * T, :]
                for k in range(ND):
                    put(base["x"] + ((i * (XC // T) + r) * ND + k) * 8, xb[:, k * T:(k + 1) * T])
                wq = jnp.concatenate([pltpu.bitcast(wq_v.bitcast(U32)[n + zs[r]], BF16) for n in range(ND)], axis=1)
                return (_dot(xb, wq) * qscale).astype(BF16).astype(F32).T

            for r in range(KR):
                broadcast_keys(KB0 + KR * i + r, kop_s[i, r:r + 1, :])
            qt = project(0)
            for r in range(XC // T):
                qt_next = project(r + 1) if r + 1 < XC // T else None
                for u in range(NU):
                    at = (i * (XC // T) + r) * NU + u
                    qu = jnp.concatenate(
                        [qt[(4 * u + j) * DH:(4 * u + j + 1) * DH] for j in range(4)], axis=1)
                    qu = jnp.concatenate([qu, jnp.zeros((KP - DH, 4 * T), F32)], axis=0)
                    norm = jnp.maximum(norm, jnp.sum(qu[:MV] * qu[:MV], axis=0, keepdims=True))
                    b11, b12, b21, b22 = qu[:HD, :2 * T], qu[:HD, 2 * T:], qu[HD:DH, :2 * T], qu[HD:DH, 2 * T:]
                    t1 = b12 - b11
                    t2 = b22 - t1
                    for p, m in enumerate([b11, b21, t2, b22 - b12, b21 - t2, t1, b22]):
                        qt_s[at, 16 * p:16 * p + HD] = m
                    qb = qu.astype(BF16)
                    qw_s[at] = _bits(qb)
                    if NPRE:
                        pre_s[at] = jnp.exp2(_dot(pltpu.bitcast(kpre_s[...], BF16)[:, :KP], qb))
                qt = qt_next
            return norm

        qnorm = lax.fori_loop(0, NXC, queries, jnp.zeros((1, 4 * T), F32))

        def rows16(g):
            return x_v[g // (XC // 16), (g % (XC // 16)) * 16:(g % (XC // 16) + 1) * 16, :]

        def keys_values():
            w_small = small_weights()
            knorm = vmax = None
            row = lax.broadcasted_iota(jnp.int32, (MV, T), 0)
            for c in range(NC):
                groups = [dict(v=vgrp, p=pgrp, m=mgrp)[src][g] for src, g in reversed(order[c])]
                kvg = _dot(w_small, jnp.concatenate([rows16(g) for g in groups], axis=0), NT)
                kt = kvg[:MV].astype(BF16).astype(F32)
                vt = kvg[MV:2 * MV].astype(BF16).astype(F32)
                sq = jnp.sum(kt * kt, axis=0, keepdims=True)
                knorm = sq if knorm is None else jnp.maximum(knorm, sq)
                vmax = jnp.abs(vt) if vmax is None else jnp.maximum(vmax, jnp.abs(vt))
                put(base["v"] + 3 * c, jnp.where(row == DH, 1.0, vt))
                kp = key_rows(kt)
                put(base["k"] + g0[c], jnp.concatenate(
                    [kp[16 * a:16 * (a + 1)] for a in reversed(range(8)) if order[c][7 - a][0] == 'm'],
                    axis=0).astype(BF16))
                gcol = jnp.broadcast_to(jax.nn.sigmoid(kvg[2 * MV:2 * MV + 1]), (T, T)).T
                for a, grp in enumerate(groups):
                    gc_s[grp // 8, (grp % 8) * 16:(grp % 8 + 1) * 16] = gcol[16 * a:16 * (a + 1)]
            return knorm, vmax

        regs = {}

        def vpu_piece(n, blk, z):
            sb, p = divmod(n, NP)
            u, b = divmod(sb, NSB)
            src = [None, 0, 0, 1, 2, None, 3][p]
            dst = [0, (0, 0), 1, 2, (1, 0), (1, 1), (0, 1)][p]

            def kept(slot):
                if (MODE[p] == "r" or (MODE[p] == "s" and slot == 2)) and slot in regs:
                    return regs[slot]
                ref = ho_s if second[sb * NP + [0, 2, 3, 5][slot]] else op_s
                return [pltpu.bitcast(ref[base["keep"] + 4 * slot + e + z], F32) for e in range(4)]

            acc = regs.get(src) if MODE[p] == 'c' else None
            chained = acc is not None
            for d in range(HD):
                qs = [jnp.broadcast_to(qt_s[blk * NU + u + z, 16 * p + d:16 * p + d + 1, j * T:(j + 1) * T], (8, T))
                      for j in range(2)]
                ks = [kb_s[b + z, p * HD + d, 8 * a:8 * (a + 1), :] for a in range(2)]
                prod = [ks[a] * qs[j] for j in range(2) for a in range(2)]
                acc = prod if acc is None else [s + m for s, m in zip(acc, prod)]
            outs = []
            if src is not None and not chained:
                acc = [s + m for s, m in zip(kept(src), acc)]
            if p == 5:
                regs[3] = [s + m for s, m in zip(kept(1), acc)]
                outs.append((base["keep"] + 12, regs[3]))
                acc = [s + m for s, m in zip(kept(2), acc)]
            if isinstance(dst, tuple):
                outs.append((base["sv"] + ((2 * sb + dst[0]) % RING) * 8 + 4 * dst[1], [jnp.exp2(v) for v in acc]))
            else:
                outs.append((base["keep"] + 4 * dst, acc))
                regs[dst] = acc
            for at, vals in outs:
                for e, v in enumerate(vals):
                    (ho_s if second[n] else op_s)[at + e + z] = _bits(v)

        for n in range(SH):
            vpu_piece(n, 0, zs[n])
        knorm, vmax = keys_values()

        vmax = jnp.max(vmax)
        safe = (jnp.max(qnorm) * jnp.max(knorm) <= 50.0 ** 2) & (vmax >= 2.0 ** -40) & (vmax <= 2.0 ** 60)

        for c in w_cp:
            c.wait()
        wg_u, wu_u, wd_u, wo_u = (r.bitcast(U32) for r in (wg_v, wu_v, wd_v, wo_v))

        def wtile(ref, n, k0, k1, z=0):
            return pltpu.bitcast(ref[n + z, k0 * (T // 2):k1 * (T // 2), :], BF16)

        def whole(ref):
            return jnp.concatenate([pltpu.bitcast(ref[n], BF16) for n in range(ref.shape[0])], axis=1)

        def mix(blk, nn, a, b):
            out_v[blk, :, nn * T:(nn + 1) * T] = (b + gc_s[blk] * (a - b)).astype(BF16)

        def out_copy(blk):
            return pltpu.make_async_copy(
                out_v.at[blk], out_hbm.at[pl.ds(pl.multiple_of(blk * T, T), T)], osems.at[blk])

        def store_heads(u, o):
            ot_s[pl.ds(4 * DH * u, 4 * DH)] = jnp.concatenate([o[:, j * T:(j + 1) * T] for j in range(4)], axis=0)

        def block(i, carry):
            state = dict(z=0, piece=SH, fetch=0)
            sv = {}
            regs.clear()
            results, later = [], []
            prev = jnp.maximum(i - 1, 0)
            nxt = jnp.minimum(i + 1, NBLK - 1)

            def zero():
                state["z"] += 1
                return zs[state["z"] % NZ]

            zl = zero()

            def flush(tm):
                while later and later[0][0] <= tm:
                    _, at, v = later.pop(0)
                    ho_s[at + zl] = _bits(v)

            def advance(tm):
                flush(tm)
                while state["piece"] < due[tm]:
                    old = [v for t, v in results if t <= tm - FWD - (FW[state['piece'] - SH] if FW else 0)]
                    if old:
                        kb_s[NSB + zero(), 0, 0:8, :] = old[-1]
                    n = state["piece"]
                    vpu_piece(n % NPIECE, i if n < NPIECE else nxt, zero())
                    state["piece"] += 1

            def vpu_weights(b, z):
                sb, half = divmod(b, 2)
                src = [ho_s if second[sb * NP + p] else op_s for p in [(1, 6), (4, 5)][half]]
                at = base["sv"] + (b % RING) * 8
                return pltpu.bitcast(jnp.concatenate(
                    [src[j // 2][pl.ds(at + 2 * j + z, 2)].reshape(16, T) for j in range(4)], axis=1), F32)

            def matmul(n, slots, dtype, w, cols=None):
                z = zero()
                ref = ho_s if prog[n][0] in second_ops else op_s
                rows = []
                for tm, at in zip(when[n], slots):
                    advance(tm)
                    rows.append(jnp.concatenate([ref[a + z] for a in at], axis=1))
                a = pltpu.bitcast(jnp.concatenate(rows, axis=0), dtype)
                r = _dot(a if cols is None else a[:, :cols], w)
                step = r.shape[0] // len(when[n])
                for g, tm in enumerate(when[n]):
                    results.append((tm, r[step * g:step * g + 8, :T]))
                return r

            def put_later(tm, at, v):
                for g in range(v.shape[0] // 8):
                    later.append((tm + 8 * g, at + g, v[8 * g:8 * (g + 1)]))
                later.sort(key=lambda e: e[0])

            def flush_region(lo, hi):
                flush(max([t for t, at, _ in later if lo <= at < hi], default=-1))

            for k in range(ND):
                put_later(2 * T + T * (k // 2), base["o"] + 16 * k, ot_s[k * T:(k + 1) * T].T)

            def x_slots(ks):
                return [[base["x"] + (i * ND + k) * 8 + g for k in ks] for g in range(8)]

            def f32_slots(region, ks):
                return [[base[region] + 16 * k + g for k in ks] for g in range(16)]

            ss = {}
            for n, op in enumerate(prog):
                kind = op[0]
                if kind == "qk":
                    u = op[1]
                    r = matmul(n, [[base["k"] + g] for g in op[2]], BF16,
                               pltpu.bitcast(qw_s[i * NU + u + zero()], BF16), KP)
                    for a, g in enumerate(op[2]):
                        ss[u, g] = r[16 * a:16 * (a + 1)]
                elif kind == "pv":
                    u, c = divmod(op[1], NC)
                    advance(when[n][0])
                    z = zero()
                    grp = [pre_s[i * NU + u + z, 16 * g:16 * (g + 1), :] if src == "p"
                           else vpu_weights(u * NB + g, z) if src == "v" else jnp.exp2(ss.pop((u, g)))
                           for src, g in reversed(order[c])]
                    acc = matmul(n, [[base["v"] + 3 * c + a] for a in range(3)], F32, jnp.concatenate(grp, axis=0))
                    if c > 0:
                        acc = acc + (acc0_s if c % 2 else acc1_s)[zero()]
                    if c < NC - 1:
                        (acc1_s if c % 2 else acc0_s)[zero()] = acc
                    else:
                        den = acc[DH:DH + 1]
                        inv = pltpu.reciprocal(den, approx=True)
                        store_heads(u, acc[:DH] * (inv * (2.0 - den * inv)))
                elif kind == "gu_b":
                    c = op[1]
                    w = jnp.concatenate(
                        [wtile(r, 2 * c + e, 4, 5, zero()) for e in range(2) for r in (wg_u, wu_u)], axis=1)
                    r = matmul(n, x_slots([4]), BF16, w)
                    z = zero()
                    for g in range(8):
                        for e in range(4):
                            gu_s[e + z, 16 * g:16 * (g + 1)] = r[16 * g:16 * (g + 1), e * T:(e + 1) * T]
                elif kind == "gate":
                    r = matmul(n, x_slots(range(4)), BF16, wtile(wg_u, op[1], 0, 4, zero()))
                    rg_s[zero()] = jnp.maximum(r + gu_s[2 * (op[1] % 2) + zero()], 0.0)
                elif kind == "up":
                    r = matmul(n, x_slots(range(4)), BF16, wtile(wu_u, op[1], 0, 4, zero()))
                    z = zero()
                    put_later(when[n][0] + DLY, base["h"] + 16 * op[1],
                              (r + gu_s[2 * (op[1] % 2) + 1 + z]) * rg_s[z])
                elif kind == "down":
                    kc, nn = op[1:]
                    flush_region(base["h"] + 64 * kc, base["h"] + 64 * (kc + 1))
                    r = matmul(n, f32_slots("h", range(4 * kc, 4 * kc + 4)), F32,
                               wtile(wd_u, nn, 4 * kc, 4 * kc + 4, zero()))
                    src, dst = (b_s, c_s) if kc == 1 else (c_s, b_s)
                    dst[nn + zero()] = r if kc == 0 else r + src[nn + zero()]
                elif kind == "oa":
                    r = matmul(n, f32_slots("o", range(4)), F32, wtile(wo_u, op[1], 0, 4, zero()))
                    z = zero()
                    mix(prev, op[1], r + b_s[ND + op[1] + z], b_s[op[1] + z])
                elif kind == "ob":
                    flush_region(base["o"], base["o"] + 16 * ND)
                    w = jnp.concatenate([wtile(wo_u, nn, 4, 5, zero()) for nn in range(4)], axis=1)
                    r = matmul(n, f32_slots("o", [4]), F32, w)
                    z = zero()
                    for g in range(16):
                        for e in range(4):
                            b_s[ND + e + z, 8 * g:8 * (g + 1)] = r[8 * g:8 * (g + 1), e * T:(e + 1) * T]
                elif kind == "oc":
                    w = wtile(wo_u, 4, 4, 5, zero())
                    advance(when[n][0])
                    b_s[ND + 4 + zero()] = jnp.concatenate(
                        [_dot(pltpu.bitcast(ho_s[pl.ds(base["o"] + 64 + 4 * a + zero(), 4)].reshape(32, T), F32), w)
                         for a in range(4)], axis=0)
            assert not later and state["piece"] == NPIECE + SH

            @pl.when(i > 0)
            def _():
                out_copy(prev).start()
            return carry

        @pl.when(safe)
        def _():
            lax.fori_loop(0, ITER or NBLK, block, 0)
            last = (ITER or NBLK) - 1
            a = _dot(ot_s[...].T, whole(wo_u))
            for nn in range(ND):
                mix(last, nn, a[:, nn * T:(nn + 1) * T], b_s[nn])
            out_copy(last).start()

        if FALLBACK:
            @pl.when(jnp.logical_not(safe))
            def _():
                def general(k_s, v_s):
                    def keys(i, carry):
                        kv = _dot(small_weights()[:2 * MV], x_v[i], NT).astype(BF16).astype(F32)
                        row = lax.broadcasted_iota(jnp.int32, (MV, XC), 0)
                        k_s[i] = key_rows(kv[:MV])
                        v_s[i] = jnp.where(row == DH, 1.0, kv[MV:])
                        return carry

                    lax.fori_loop(0, NXC, keys, 0)

                    def rows(i, carry):
                        def unit(u, carry):
                            q = pltpu.bitcast(qw_s[i * NU + u], BF16)

                            def chunk(c, carry):
                                m, acc = carry
                                s = _dot(k_s[c][:, :KP], q)
                                m_new = jnp.maximum(m, jnp.max(s, axis=0, keepdims=True))
                                return m_new, acc * jnp.exp2(m - m_new) + _dot(v_s[c], jnp.exp2(s - m_new))

                            _, acc = lax.fori_loop(
                                0, NXC, chunk, (jnp.full((1, 4 * T), -jnp.inf, F32), jnp.zeros((MV, 4 * T), F32)))
                            o = acc[:DH] / acc[DH:DH + 1]
                            ot_s[pl.ds(pl.multiple_of(4 * DH * u, 4 * DH), 4 * DH)] = jnp.concatenate(
                                [o[:, j * T:(j + 1) * T] for j in range(4)], axis=0)
                            return carry

                        lax.fori_loop(0, NU, unit, 0)
                        x = pltpu.bitcast(jnp.concatenate(
                            [op_s[pl.ds(base["x"] + (i * ND + k) * 8, 8)].reshape(T // 2, T) for k in range(ND)],
                            axis=1), BF16)
                        h = jnp.maximum(_dot(x, whole(wg_u)), 0.0) * _dot(x, whole(wu_u))
                        a, b = _dot(ot_s[...].T, whole(wo_u)), _dot(h, whole(wd_u))
                        for nn in range(ND):
                            mix(i, nn, a[:, nn * T:(nn + 1) * T], b[:, nn * T:(nn + 1) * T])
                        out_copy(i).start()
                        return carry

                    lax.fori_loop(0, ITER or NBLK, rows, 0)

                pl.run_scoped(general, pltpu.VMEM((NXC, XC, T), F32), pltpu.VMEM((NXC, MV, XC), F32))

        for i in range(ITER or NBLK):
            out_copy(i).wait()

    anyspec = pl.BlockSpec(memory_space=pl.ANY)
    V = pltpu.VMEM
    call = pl.pallas_call(
        kernel,
        out_shape=jax.ShapeDtypeStruct((S, D), BF16),
        in_specs=[anyspec] * 8 + [pl.BlockSpec(memory_space=V)],
        out_specs=anyspec,
        scratch_shapes=[
            V((NXC, XC, D), BF16), V((ND, D, T), BF16), V((DH, D), BF16), V((DH, D), BF16),
            V((ND, D, T), BF16), V((NF, D, T), BF16), V((NF, D, T), BF16), V((ND, F, T), BF16),
            V((top, 8, T), U32), V((top2, 8, T), U32), V((NSB + 1, (KB0 + NXC * KR + 1) // 2 * 2, 16, T), F32), V((MV, XC), F32),
            V((NXC, KR, pl.cdiv(NSB, 8) * T), F32), V((8 * max(NPRE, 1), T), U32),
            V((NBLK * NU, NP * 16, 2 * T), F32), V((NBLK * NU, KP // 2, 4 * T), U32),
            V((NBLK * NU, 16 * max(NPRE, 1), 4 * T), F32),
            V((NBLK, T, T), F32), V((D, T), F32), V((1, MV, 4 * T), F32), V((1, MV, 4 * T), F32),
            V((4, T, T), F32), V((1, T, T), F32), V((2 * ND, T, T), F32), V((ND, T, T), F32),
            V((NBLK, T, D), BF16),
            pltpu.SMEM((NZ,), jnp.int32),
            pltpu.SemaphoreType.DMA((NXC,)), pltpu.SemaphoreType.DMA((2 + ND,)),
            pltpu.SemaphoreType.DMA((2 * NF + 2 * ND,)), pltpu.SemaphoreType.DMA((NBLK,)),
        ],
        compiler_params=pltpu.CompilerParams(vmem_limit_bytes=100 * 2**20, flags=flags),
        name=name,
    )

    @jax.jit
    def fn(A_x, A_wq, A_wk, A_wv, A_wo, B_x, B_W_gate, B_W_up, B_W_down, gate_w):
        out = call(A_x.reshape(S, D), A_wq, A_wk.T, A_wv.T, A_wo, B_W_gate, B_W_up, B_W_down, gate_w)
        return out.reshape(1, S, D)

    return fn


_fn = make()


@jax.jit
def pallas_gated_mix__grouped_kv_mqa__glu_gated_reglu__prompt_kernel(
    A_x, A_wq, A_wk, A_wv, A_wo, B_x, B_W_gate, B_W_up, B_W_down, gate_w):
    return _fn(A_x, A_wq, A_wk, A_wv, A_wo, B_x, B_W_gate, B_W_up, B_W_down, gate_w)
```

```python
import math

import jax
import jax.numpy as jnp
from jax import lax
import jax.experimental.pallas as pl
import jax.experimental.pallas.tpu as pltpu

F32, BF16, U32 = jnp.float32, jnp.bfloat16, jnp.uint32
NN = (((1,), (0,)), ((), ()))
NT = (((1,), (1,)), ((), ()))

S, D, H, F = 2048, 640, 32, 1536
T = 128
DH = D // H
HD = DH // 2
NBLK = NC = S // T
NU = H // 4
MV = 24
KP = 32
ND, NF = D // T, F // T
XC = 512
NXC = S // XC
FS = F // (NXC - 1)
QSCALE = DH ** -0.5 * math.log2(math.e)
SCORE_BOUND = 50.0

N_VPU, N_PRE = 28, 4
NPAIR = N_VPU // 2
NP = 7
G_MXU = [int(ch) for ch in "5675675675676567"]
G_PRE = [int(c % 4 == 2) for c in range(NC)]
G_VPU = [8 - a - b for a, b in zip(G_MXU, G_PRE)]
assert sum(G_VPU) == N_VPU and sum(G_PRE) == N_PRE
VPU_0, PRE_0, MXU_0 = ([sum(v[:c]) for c in range(NC)] for v in (G_VPU, G_PRE, G_MXU))
VPU_GROUPS = [(b // 16) * 16 + (b % 2) * 8 + (b % 16) // 2 for b in range(N_VPU)]
PRE_GROUPS = [g for g in range(S // 16) if g not in VPU_GROUPS][:N_PRE]
MXU_GROUPS = [g for g in range(S // 16) if g not in VPU_GROUPS][N_PRE:]
assert max(VPU_GROUPS + PRE_GROUPS) < XC // 16

RING = 16
AT_P = 0
AT_KEEP = AT_P + 8 * RING
AT_K = AT_H = AT_KEEP + 16
AT_V = AT_K + 2 * len(MXU_GROUPS)
AT_X = AT_V + 3 * NC
AT_O = AT_H + 16 * NF
N_X = 8 * ND * NBLK
AT_W = dict(g=0, u=D * F // 2048, d=2 * D * F // 2048, o=3 * D * F // 2048, x=(3 * F + D) * D // 2048)
NZ = 64
KB_FIRST = 2
KB_STEP = (NP * HD - KB_FIRST) // NXC
assert KB_FIRST + NXC * KB_STEP == NP * HD and FS == XC


def _mxu_programme():
    latency, max_groups = 152, 8
    downs = [("down", kc, n) for kc in range(NF // 4) for n in range(ND)]
    dense = []
    for c in range(NF // 2):
        dense.append(("gu", c))
        if c in (2, 4):
            dense += downs[:ND] if c == 2 else downs[ND:2 * ND - 1]
        dense += [("gate", 2 * c), ("up", 2 * c), ("gate", 2 * c + 1), ("up", 2 * c + 1)]
        if c == 0:
            dense += [("ob",)] + [("oa", n) for n in range(4)] + [("oc",), ("oa", 4)]
    dense += downs[2 * ND - 1:]
    final = dense.pop()
    groups = [(t, a) for t in range(NU * NC) for a in range(G_MXU[t % NC])]
    prog, waiting, now, g, w = [], [], 0, 0, 0
    while g < len(groups) or waiting:
        if waiting and now - waiting[0][1] >= (latency if g < len(groups) else T):
            prog.append(("pv", waiting.pop(0)[0]))
            now += MV
            quiet = len(waiting) <= 1 and g < len(groups) and groups[g][1] <= 1
            while quiet and w < len(dense) and (
                    prog[-1][0] == "pv" and dense[w][0] != "oc" if waiting else
                    (w + 0.7) * len(groups) <= g * len(dense) or dense[w][0] == "oc"):
                prog.append(dense[w])
                now += 32 if dense[w][0] == "oc" else T
                w += 1
        elif g < len(groups):
            t, a = groups[g]
            if prog and prog[-1][:2] == ("qk", t // NC) and len(prog[-1][2]) < max_groups:
                prog[-1][2].append(MXU_0[t % NC] + a)
            else:
                prog.append(("qk", t // NC, [MXU_0[t % NC] + a]))
            g += 1
            now += 16
            if a == G_MXU[t % NC] - 1:
                waiting.append((t, now))
        else:
            if w < len(dense):
                prog.append(dense[w])
                w += 1
            now += T
    prog += dense[w:] + [final]

    when, now = [], 0
    for op in prog:
        if op[0] == "qk":
            n, cycles = 2 * len(op[2]), 8
        else:
            n, cycles = dict(pv=(3, 8), oc=(1, 32), down=(16, 8), oa=(16, 8), ob=(16, 8)).get(op[0], (8, 16))
        when.append([now + cycles * a for a in range(n)])
        now += cycles * n
    return prog, when


PROG, WHEN = _mxu_programme()
READS_HO = ("down", "oa", "ob", "oc")
NPIECE = NU * NPAIR * NP
AHEAD = 4 * NP
START_AFTER = 212
H_DELAY = 150


def _pin_pieces():
    reads = [(tm, op[0]) for op, row in zip(PROG, WHEN) for tm in row]
    pin, in_ho, a = [], {}, 0
    for n in range(NPIECE):
        goal = (n + 1) * (reads[-1][0] + 1) / NPIECE - 1
        while a + 1 < len(reads) and reads[a + 1][0] - goal <= goal - reads[a][0]:
            a += 1
        pin.append(reads[a][0])
        in_ho[(n + AHEAD) % NPIECE] = reads[a][1] in READS_HO
    return pin, in_ho


PIN, IN_HO = _pin_pieces()


def _dot(a, b, dims=NN):
    return lax.dot_general(a, b, dims, preferred_element_type=F32)


def _round(v):
    return v.astype(BF16).astype(F32)


def _side_by_side(v):
    n, r, c = v.shape
    return jnp.concatenate(lax.split(v.reshape(n * r, c), [r] * n), axis=1)


def _put(ref, at, v):
    v = pltpu.bitcast(v, U32)
    ref[pl.ds(at, v.shape[0] // 8)] = v.reshape(v.shape[0] // 8, 8, T)


def _key_rows(kt):
    return jnp.concatenate([kt, jnp.zeros((T - MV, kt.shape[1]), F32)], axis=0).T


def _kernel(x_hbm, wq_hbm, wkt_hbm, wvt_hbm, wo_hbm, wg_hbm, wu_hbm, wd_hbm, gw_hbm, out_hbm,
            x_v, wq_v, wo_v, gu_v, wd_v, w_s, op_s, ho_s, kb_s, kop_s, kpre_s, qt_s, qv_s, qw_s, pre_s,
            gc_s, ot_s, acc0_s, acc1_s, part_s, relu_s, b_s, c_s, out_v, wkt_v, wvt_v, gw_v,
            zs, sems, osems):
    copies = []

    def copy(src, dst):
        copies.append(pltpu.make_async_copy(src, dst, sems.at[len(copies)]))
        return copies[-1]

    small = [copy(wkt_hbm, wkt_v), copy(wvt_hbm, wvt_v), copy(gw_hbm, gw_v)]
    wq_copy = copy(wq_hbm, wq_v.at[0])
    stages = [[copy(x_hbm.at[pl.ds(i * XC, XC)], x_v.at[i])] for i in range(NXC)] + [[copy(wd_hbm, wd_v)]]
    for i in range(1, NXC):
        cols = pl.ds((i - 1) * FS, FS)
        lo, hi = (16 * (e * (D // 16) // (NXC - 1)) for e in (i - 1, i))
        stages[i] += [copy(wg_hbm.at[:, cols], gu_v.at[i, 0]), copy(wu_hbm.at[:, cols], gu_v.at[i, 1]),
                      copy(wo_hbm.at[pl.ds(lo, hi - lo)], wo_v.at[pl.ds(lo, hi - lo)])]
    for c in small + stages[0]:
        c.start()
    ot_s[...] = jnp.zeros(ot_s.shape, F32)
    b_s[...] = jnp.zeros(b_s.shape, F32)
    for i in range(NZ):
        zs[i] = 0
    for c in small:
        c.wait()
    wq_copy.start()
    gu_v[0] = jnp.zeros(gu_v.shape[1:], BF16)

    def small_weights():
        pad = jnp.zeros((MV - DH, D), F32)
        gw = gw_v[...].astype(F32).reshape(1, D)
        return jnp.concatenate([wkt_v[...].astype(F32), pad, wvt_v[...].astype(F32), pad,
                                jnp.broadcast_to(gw, (8, D))], axis=0)

    stages[0][0].wait()
    kt = _round(_dot(small_weights()[:MV], x_v[0], NT))
    first = jnp.concatenate([kt[:, :T], kt[:, 2 * T:3 * T]], axis=1)
    other = jnp.concatenate([kt[:, T:2 * T], kt[:, 3 * T:]], axis=1)
    a11, a12, a21, a22 = first[:HD], first[HD:DH], other[:HD], other[HD:DH]
    s1 = a21 + a22
    s2 = s1 - a11
    kop = jnp.concatenate([a11, a12, s2, a11 - a21, a22, s1, a12 - s2], axis=0)
    for i in range(NXC):
        kop_s[i] = kop[KB_FIRST + KB_STEP * i:KB_FIRST + KB_STEP * (i + 1)]

    def broadcast_keys(at, row):
        for c in range(2):
            n = min(8, NPAIR - 8 * c)
            col = jnp.broadcast_to(row[:, c * T:(c + 1) * T], (T, T)).T
            kb_s[8 * c:8 * c + n, at] = col[:16 * n].reshape(n, 16, T)

    k0 = _key_rows(kt)
    kpre_s[...] = pltpu.bitcast(
        jnp.concatenate([k0[16 * g:16 * (g + 1)] for g in PRE_GROUPS], axis=0).astype(BF16), U32)
    for r in range(KB_FIRST):
        broadcast_keys(r, kop[r:r + 1])
    wq_copy.wait()
    for c in stages[1]:
        c.start()

    def queries(i, norm):
        for e in range(1, NXC):
            @pl.when(i == e)
            def _():
                for c in stages[e + 1]:
                    c.start()
                for c in stages[e]:
                    c.wait()

        def project(r):
            xb = x_v[i, r * T:(r + 1) * T, :]
            xu = pltpu.bitcast(xb, U32)
            xu = jnp.concatenate(
                [xu[8 * g:8 * (g + 1), k * T:(k + 1) * T] for g in range(8) for k in range(ND)], axis=0)
            at = (i * (XC // T) + r) * 8 * ND
            _put(op_s, AT_X + at, xu)
            _put(w_s, AT_W["x"] + at, xu)
            for e, key in enumerate("gu"):
                _put(w_s, AT_W[key] + (jnp.maximum(i - 1, 0) * (FS // T) + r) * (D // 16),
                     gu_v[i, e, :, r * T:(r + 1) * T])
            return _round(_dot(xb, wq_v[zs[r]]) * QSCALE).T

        for r in range(KB_STEP):
            broadcast_keys(KB_FIRST + KB_STEP * i + r, kop_s[i, r:r + 1, :])
        qt = project(0)
        for r in range(XC // T):
            qt_next = project(r + 1) if r + 1 < XC // T else None
            blk = i * (XC // T) + r
            for u in range(NU):
                qu = jnp.concatenate([qt[(NU * j + u) * DH:(NU * j + u + 1) * DH] for j in range(4)], axis=1)
                qu = jnp.concatenate([qu, jnp.zeros((KP - DH, 4 * T), F32)], axis=0).astype(BF16)
                qw_s[blk * NU + u] = pltpu.bitcast(qu, U32)
                pre_s[blk * NU + u] = jnp.exp2(_dot(pltpu.bitcast(kpre_s[...], BF16)[:, :KP], qu))
            qt_s[r] = qt
            heads = [jnp.stack([qt_s[r, pl.ds(NU * DH * j + d, NU, stride=DH), :] for d in range(DH)])
                     for j in range(4)]
            for m in heads:
                norm = jnp.maximum(norm, jnp.sum(m * m, axis=0))
            left, right = jnp.concatenate(heads[:2], axis=2), jnp.concatenate(heads[2:], axis=2)
            b11, b12, b21, b22 = left[:HD], right[:HD], left[HD:], right[HD:]
            t1 = b12 - b11
            t2 = b22 - t1
            qv_s[blk] = jnp.concatenate([b11, b21, t2, b22 - b12, b21 - t2, t1, b22], axis=0)
            qt = qt_next
        return norm

    q_norm = lax.fori_loop(0, NXC, queries, jnp.zeros((NU, T), F32))

    held = {}

    def vpu_product(n, blk, z):
        pair, p = divmod(n, NP)
        u, b = divmod(pair, NPAIR)
        out = ho_s if IN_HO[n] else op_s

        def kept(slot):
            if p in (1, 3, 6):
                return held[slot]
            ref = ho_s if IN_HO[pair * NP + (0, 2, 3)[slot]] else op_s
            return pltpu.bitcast(ref[pl.ds(AT_KEEP + 4 * slot + z, 4)].reshape(32, T), F32)

        acc, last = None, None
        k_at, q_at = b + z, blk + z
        for d in (p * HD, p * HD + HD // 2):
            rows = pl.ds(d, HD // 2)
            qs = jnp.concatenate([jnp.broadcast_to(qv_s[q_at, rows, u:u + 1, j * T:(j + 1) * T],
                                                   (HD // 2, 16, T)) for j in range(2)], axis=1)
            ks = kb_s[k_at, rows]
            ks = jnp.concatenate([ks, ks], axis=1)
            for k, q in zip(*(lax.split(v.reshape(16 * HD, T), [32] * (HD // 2)) for v in (ks, qs))):
                prod = k * q
                if last is not None:
                    acc = last if acc is None else acc + last
                last = prod
        acc = acc + last
        if p == 5:
            held[3] = acc + kept(1)
            acc = acc + kept(2)
            _put(out, AT_KEEP + 12 + z, held[3])
        elif p > 0:
            acc = acc + kept((None, 0, 0, 1, 2, None, 3)[p])
        if p in (0, 2, 3):
            slot = (0, None, 1, 2)[p]
            _put(out, AT_KEEP + 4 * slot + z, acc)
            held[slot] = acc
        else:
            group, half = {1: (0, 0), 4: (1, 0), 5: (1, 1), 6: (0, 1)}[p]
            _put(out, AT_P + (2 * pair + group) % RING * 8 + 4 * half + z, jnp.exp2(acc))

    stages[NXC][0].wait()
    repack = [(AT_W[key] + n * (src.shape[0] // 16) + 8 * k, src, n, k)
              for src, key in ((wd_v, "d"), (wo_v, "o"))
              for n in range(src.shape[1] // T) for k in range(src.shape[0] // T)]
    w_small = small_weights()
    ones_row = lax.broadcasted_iota(jnp.int32, (MV, T), 0) == DH
    k_norm = v_max = None
    for c in range(NC):
        groups = (PRE_GROUPS[PRE_0[c]:PRE_0[c] + G_PRE[c]] + VPU_GROUPS[VPU_0[c]:VPU_0[c] + G_VPU[c]]
                  + MXU_GROUPS[MXU_0[c]:MXU_0[c] + G_MXU[c]][::-1])
        z = zs[c]
        xt = jnp.concatenate([w_s[pl.ds(AT_W["x"] + ND * g + z, ND)] for g in groups], axis=1)
        kvg = _dot(w_small, pltpu.bitcast(_side_by_side(xt), BF16), NT)
        for n in range(c * AHEAD // (NC - 1), min((c + 1) * AHEAD // (NC - 1), AHEAD)):
            vpu_product(n, 0, zs[n])
        for at, src, n, k in repack[c::NC]:
            _put(w_s, at, src[k * T:(k + 1) * T, n * T:(n + 1) * T])
        kt, vt = _round(kvg[:MV]), _round(kvg[MV:2 * MV])
        sq = jnp.sum(kt * kt, axis=0, keepdims=True)
        k_norm = sq if k_norm is None else jnp.maximum(k_norm, sq)
        v_max = jnp.abs(vt) if v_max is None else jnp.maximum(v_max, jnp.abs(vt))
        kp = _key_rows(kt)
        _put(op_s, AT_V + 3 * c, jnp.where(ones_row, 1.0, vt))
        _put(op_s, AT_K + 2 * MXU_0[c], jnp.concatenate(
            [kp[16 * a:16 * (a + 1)] for a in reversed(range(8 - G_MXU[c], 8))], axis=0))
        gate = jnp.broadcast_to(jax.nn.sigmoid(kvg[2 * MV:2 * MV + 1]), (T, T)).T
        for a, g in enumerate(groups):
            gc_s[g // 8, (g % 8) * 16:(g % 8 + 1) * 16] = gate[16 * a:16 * (a + 1)]

    v_max = jnp.max(v_max)
    bounded = ((jnp.max(q_norm) * jnp.max(k_norm) <= SCORE_BOUND ** 2)
               & (v_max >= 2.0 ** -40) & (v_max <= 2.0 ** 60))

    def weights(key, n, k0, k1, z):
        at = AT_W[key] + n * (F // 16 if key == "d" else D // 16) + 8 * k0 + z
        return pltpu.bitcast(w_s[pl.ds(at, 8 * (k1 - k0))].reshape(64 * (k1 - k0), T), BF16)

    def store_heads(u, o):
        for j in range(4):
            ot_s[(NU * j + u) * DH:(NU * j + u + 1) * DH] = o[:, j * T:(j + 1) * T]

    def mix(blk, n, a, b):
        out_v[blk, :, n * T:(n + 1) * T] = (b + gc_s[blk] * (a - b)).astype(BF16)

    def out_copy(blk):
        return pltpu.make_async_copy(
            out_v.at[blk], out_hbm.at[pl.ds(pl.multiple_of(blk * T, T), T)], osems.at[blk])

    def block(i, carry):
        count = dict(zero=0, product=0)
        held.clear()
        issued, later, scores = [], [], {}
        following = jnp.minimum(i + 1, NBLK - 1)
        previous = jnp.maximum(i - 1, 0)

        def zero():
            count["zero"] += 1
            return zs[count["zero"] % NZ]

        z_later = zero()

        def flush(tm):
            while later and later[0][0] <= tm:
                _, at, v = later.pop(0)
                _put(ho_s, at + z_later, v)

        def put_later(tm, first, stride, v):
            for g in range(v.shape[0] // 8):
                later.append((tm + 8 * g, first + stride * g, v[8 * g:8 * (g + 1)]))
            later.sort(key=lambda e: e[0])

        def flush_slots(lo, hi):
            flush(max([tm for tm, at, _ in later if lo <= at < hi], default=-1))

        def advance(tm):
            flush(tm)
            while count["product"] < NPIECE and PIN[count["product"]] <= tm:
                n = count["product"] + AHEAD
                old = [e for e in issued[-96:] if e[0] <= tm - START_AFTER]
                if old:
                    _, r, at = old[-1]
                    kb_s[NPAIR + zero(), 0, 0:8, :] = r[at:at + 8, r.shape[1] - T:]
                vpu_product(n % NPIECE, i if n < NPIECE else following, zero())
                count["product"] += 1

        def matmul(n, first, stride, width, dtype, w, cols=None):
            ref = ho_s if PROG[n][0] in READS_HO else op_s
            first = first + zero()
            rows = []
            for g, tm in enumerate(WHEN[n]):
                advance(tm)
                rows.append(ref[pl.ds(first + stride * g, width)])
            a = pltpu.bitcast(_side_by_side(jnp.concatenate(rows, axis=1)), dtype)
            r = _dot(a if cols is None else a[:, :cols], w)
            issued.extend((tm, r, r.shape[0] // len(WHEN[n]) * g) for g, tm in enumerate(WHEN[n]))
            return r

        for k in range(ND):
            put_later(2 * T + T * (k // 2), AT_O + k, ND, ot_s[k * T:(k + 1) * T].T)
        x_at = AT_X + i * (8 * ND)
        for n, op in enumerate(PROG):
            kind = op[0]
            if kind == "qk":
                q = pltpu.bitcast(qw_s[i * NU + op[1] + zero()], BF16)
                r = matmul(n, AT_K + 2 * op[2][0], 1, 1, F32, q, KP)
                for a, g in enumerate(op[2]):
                    scores[op[1], g] = r[16 * a:16 * (a + 1)]
            elif kind == "pv":
                u, c = divmod(op[1], NC)
                z = zero()
                p = [pre_s[i * NU + u + z, 16 * g:16 * (g + 1), :] for g in range(PRE_0[c], PRE_0[c] + G_PRE[c])]
                for b in range(u * N_VPU + VPU_0[c], u * N_VPU + VPU_0[c] + G_VPU[c]):
                    made_by = [b // 2 * NP + e for e in ((1, 6), (4, 5))[b % 2]]
                    assert max(made_by) < count["product"] + AHEAD <= (b + RING) // 2 * NP + 1
                    at = AT_P + b % RING * 8 + z
                    both = [(ho_s if IN_HO[m] else op_s)[pl.ds(at + 4 * e, 4)] for e, m in enumerate(made_by)]
                    p.append(pltpu.bitcast(_side_by_side(jnp.concatenate(both, axis=0).reshape(4, 16, T)), F32))
                p.append(jnp.exp2(jnp.concatenate(
                    [scores.pop((u, MXU_0[c] + a)) for a in reversed(range(G_MXU[c]))], axis=0)))
                acc = matmul(n, AT_V + 3 * c, 1, 1, F32, jnp.concatenate(p, axis=0))
                if c > 0:
                    acc = acc + (acc0_s if c % 2 else acc1_s)[zero()]
                if c < NC - 1:
                    (acc1_s if c % 2 else acc0_s)[zero()] = acc
                else:
                    den = acc[DH:DH + 1]
                    inv = pltpu.reciprocal(den, approx=True)
                    store_heads(u, acc[:DH] * (inv * (2.0 - den * inv)))
            elif kind == "gu":
                z = zero()
                w = jnp.concatenate([weights(key, 2 * op[1] + e, 4, 5, z) for e in range(2) for key in "gu"], axis=1)
                part_s[z] = matmul(n, x_at + 4, ND, 1, BF16, w)
            elif kind == "gate":
                e = 2 * (op[1] % 2)
                r = matmul(n, x_at, ND, 4, BF16, weights("g", op[1], 0, 4, zero()))
                z = zero()
                relu_s[z] = jnp.maximum(r + part_s[z, :, e * T:(e + 1) * T], 0.0)
            elif kind == "up":
                e = 2 * (op[1] % 2) + 1
                r = matmul(n, x_at, ND, 4, BF16, weights("u", op[1], 0, 4, zero()))
                z = zero()
                put_later(WHEN[n][0] + H_DELAY, AT_H + 64 * (op[1] // 4) + op[1] % 4, 4,
                          (r + part_s[z, :, e * T:(e + 1) * T]) * relu_s[z])
            elif kind == "down":
                kc, col = op[1:]
                flush_slots(AT_H + 64 * kc, AT_H + 64 * (kc + 1))
                r = matmul(n, AT_H + 64 * kc, 4, 4, F32, weights("d", col, 4 * kc, 4 * kc + 4, zero()))
                src, dst = (b_s, c_s) if kc == 1 else (c_s, b_s)
                dst[col + zero()] = r if kc == 0 else r + src[col + zero()]
            elif kind == "ob":
                flush_slots(AT_O, AT_O + 16 * ND)
                z = zero()
                w = jnp.concatenate([weights("o", col, 4, 5, z) for col in range(4)], axis=1)
                part_s[z] = matmul(n, AT_O + 4, ND, 1, F32, w)
            elif kind == "oc":
                w = weights("o", 4, 4, 5, zero())
                advance(WHEN[n][0])
                z = zero()
                relu_s[z] = jnp.concatenate([_dot(pltpu.bitcast(jnp.concatenate(
                    [ho_s[AT_O + 4 + ND * g + z] for g in range(4 * a, 4 * a + 4)], axis=0), F32), w)
                    for a in range(4)], axis=0)
            else:
                col = op[1]
                r = matmul(n, AT_O, ND, 4, F32, weights("o", col, 0, 4, zero()))
                z = zero()
                r = r + (part_s[z, :, col * T:(col + 1) * T] if col < 4 else relu_s[z])
                mix(previous, col, r, b_s[col + z])
        assert not later and count["product"] == NPIECE

        @pl.when(i > 0)
        def _():
            out_copy(previous).start()

        return carry

    @pl.when(bounded)
    def _():
        lax.fori_loop(0, NBLK, block, 0)
        a = _dot(ot_s[...].T, wo_v[...])
        for n in range(ND):
            mix(NBLK - 1, n, a[:, n * T:(n + 1) * T], b_s[n])
        out_copy(NBLK - 1).start()

    def general(k_s, v_s, o_s):
        def keys(i, carry):
            kv = _round(_dot(small_weights()[:2 * MV], x_v[i], NT))
            row = lax.broadcasted_iota(jnp.int32, (MV, XC), 0)
            k_s[i] = _key_rows(kv[:MV])
            v_s[i] = jnp.where(row == DH, 1.0, kv[MV:])
            return carry

        lax.fori_loop(0, NXC, keys, 0)

        def rows(i, carry):
            def unit(u, carry):
                q = pltpu.bitcast(qw_s[i * NU + u], BF16)

                def chunk(c, carry):
                    m, acc = carry
                    s = _dot(k_s[c][:, :KP], q)
                    m_new = jnp.maximum(m, jnp.max(s, axis=0, keepdims=True))
                    return m_new, acc * jnp.exp2(m - m_new) + _dot(v_s[c], jnp.exp2(s - m_new))

                lowest = jnp.full((1, 4 * T), float(jnp.finfo(F32).min), F32)
                _, acc = lax.fori_loop(0, NXC, chunk, (lowest, jnp.zeros((MV, 4 * T), F32)))
                o_s[u] = acc / acc[DH:DH + 1]
                return carry

            lax.fori_loop(0, NU, unit, 0)
            for u in range(NU):
                store_heads(u, o_s[u, :DH])
            x = x_v[i // (XC // T), pl.ds(pl.multiple_of(i % (XC // T) * T, T), T), :]
            h = jnp.concatenate([jnp.maximum(_dot(x, gu_v[e, 0]), 0.0) * _dot(x, gu_v[e, 1])
                                 for e in range(1, NXC)], axis=1)
            a, b = _dot(ot_s[...].T, wo_v[...]), _dot(h, wd_v[...])
            for n in range(ND):
                mix(i, n, a[:, n * T:(n + 1) * T], b[:, n * T:(n + 1) * T])
            out_copy(i).start()
            return carry

        lax.fori_loop(0, NBLK, rows, 0)

    @pl.when(jnp.logical_not(bounded))
    def _():
        pl.run_scoped(general, pltpu.VMEM((NXC, XC, T), F32), pltpu.VMEM((NXC, MV, XC), F32),
                      pltpu.VMEM((NU, MV, 4 * T), F32))

    for i in range(NBLK):
        out_copy(i).wait()


@jax.jit
def pallas_gated_mix__grouped_kv_mqa__glu_gated_reglu__prompt_kernel(
    A_x: jax.Array,
    A_wq: jax.Array,
    A_wk: jax.Array,
    A_wv: jax.Array,
    A_wo: jax.Array,
    B_x: jax.Array,
    B_W_gate: jax.Array,
    B_W_up: jax.Array,
    B_W_down: jax.Array,
    gate_w: jax.Array,
):
    del B_x
    vmem = pltpu.VMEM
    anywhere = pl.BlockSpec(memory_space=pl.ANY)
    out = pl.pallas_call(
        _kernel,
        out_shape=jax.ShapeDtypeStruct((S, D), BF16),
        in_specs=[anywhere] * 9,
        out_specs=anywhere,
        scratch_shapes=[
            vmem((NXC, XC, D), BF16),
            vmem((1, D, D), BF16),
            vmem((D, D), BF16),
            vmem((NXC, 2, D, FS), BF16),
            vmem((F, D), BF16),
            vmem((AT_W["x"] + N_X, 8, T), U32),
            vmem((AT_X + N_X, 8, T), U32),
            vmem((AT_O + 16 * ND, 8, T), U32),
            vmem((NPAIR + 1, NP * HD, 16, T), F32),
            vmem((NXC, KB_STEP, 2 * T), F32),
            vmem((8 * N_PRE, T), U32),
            vmem((XC // T, D, T), F32),
            vmem((NBLK, NP * HD, NU, 2 * T), F32),
            vmem((NBLK * NU, KP // 2, 4 * T), U32),
            vmem((NBLK * NU, 16 * N_PRE, 4 * T), F32),
            vmem((NBLK, T, T), F32),
            vmem((D, T), F32),
            vmem((1, MV, 4 * T), F32),
            vmem((1, MV, 4 * T), F32),
            vmem((1, T, 4 * T), F32),
            vmem((1, T, T), F32),
            vmem((ND, T, T), F32),
            vmem((ND, T, T), F32),
            vmem((NBLK, T, D), BF16),
            vmem((DH, D), BF16),
            vmem((DH, D), BF16),
            vmem((D,), BF16),
            pltpu.SMEM((NZ,), jnp.int32),
            pltpu.SemaphoreType.DMA((4 * NXC + 2,)),
            pltpu.SemaphoreType.DMA((NBLK,)),
        ],
        compiler_params=pltpu.CompilerParams(vmem_limit_bytes=100 * 2**20),
        name="gated_mix_mqa_reglu",
    )(A_x.reshape(S, D), A_wq, A_wk.T, A_wv.T, A_wo, B_W_gate, B_W_up, B_W_down, gate_w)
    return out.reshape(1, S, D)
```
